```python
import jax
import jax.numpy as jnp

def _softmax(x, axis=-1):
    return jax.nn.softmax(x, axis=axis)

def _gelu(x):
    return jax.nn.gelu(x, approximate=True)

def _silu(x):
    return jax.nn.silu(x)

def _sigmoid(x):
    return jax.nn.sigmoid(x)

def _layernorm(x, axis=-1, eps=1e-05):
    m = jnp.mean(x, axis=axis, keepdims=True)
    v = jnp.var(x, axis=axis, keepdims=True)
    return (x - m) / jnp.sqrt(v + eps)

def _scatter_add(tgt, idx, src, axis=0):
    return tgt.at[idx].add(src)

def _segment_sum(src, seg, n):
    return jax.ops.segment_sum(src, seg, n)

class _Rng:

    def __init__(self, key):
        self._k = key

    def _next(self):
        self._k, sub = jax.random.split(self._k)
        return sub

    def normal(self, shape):
        return jax.random.normal(self._next(), shape, dtype=jnp.bfloat16)

    def randint(self, lo, hi, shape):
        return jax.random.randint(self._next(), shape, lo, hi, dtype=jnp.int32)

    def uniform(self, shape, lo=0.0, hi=1.0):
        return jax.random.uniform(self._next(), shape, jnp.bfloat16, lo, hi)

    def permutation(self, n):
        return jax.random.permutation(self._next(), n)
kernel_name = 'interleave_layers__memory_aug_recurrent_mem_tr__sliding_local_dilated__prompt'

def setup_inputs():
    _rng = _Rng(jax.random.key(int.from_bytes(__import__("os").urandom(4), "little")))
    _w = lambda a: (lambda t: t.astype(jnp.bfloat16) if jnp.issubdtype(t.dtype, jnp.floating) else t)(jnp.asarray(a))

    def _A_setup():
        B, S, Dm = (1, 2048, 640)
        H, Dh = (32, 192)
        M, seg = (8, 32)
        seg = min(seg, S)
        S = S // seg * seg
        return {'x': _w((lambda *s: _rng.normal(s) * 0.05)(B, S, Dm)), 'mem0': _w((lambda *s: _rng.normal(s) * 0.05)(B, M, Dm)), 'Wq': _w((lambda *s: _rng.normal(s) * 0.05)(Dm, H, Dh) * Dm ** (-0.5)), 'Wk': _w((lambda *s: _rng.normal(s) * 0.05)(Dm, H, Dh) * Dm ** (-0.5)), 'Wv': _w((lambda *s: _rng.normal(s) * 0.05)(Dm, H, Dh) * Dm ** (-0.5)), 'Wo': _w((lambda *s: _rng.normal(s) * 0.05)(H, Dh, Dm) * (H * Dh) ** (-0.5)), 'seg_len': seg}
    _A_in = _A_setup()

    def _B_setup():
        B, S, D = (1, 2048, 640)
        return {'x': _w((lambda *s: _rng.normal(s) * 0.05)(B, S, D)), 'wqkv': _w((lambda *s: _rng.normal(s) * 0.05)(D, 3 * D)), 'wo': _w((lambda *s: _rng.normal(s) * 0.05)(D, D))}
    _B_in = _B_setup()
    return {'A_x': _A_in['x'], 'A_mem0': _A_in['mem0'], 'A_Wq': _A_in['Wq'], 'A_Wk': _A_in['Wk'], 'A_Wv': _A_in['Wv'], 'A_Wo': _A_in['Wo'], 'A_seg_len': _A_in['seg_len'], 'B_x': _B_in['x'], 'B_wqkv': _B_in['wqkv'], 'B_wo': _B_in['wo']}

def reference(A_x, A_mem0, A_Wq, A_Wk, A_Wv, A_Wo, A_seg_len, B_x, B_wqkv, B_wo):

    def _A_ref(x, mem0, Wq, Wk, Wv, Wo, seg_len):
        B, S, Dm = x.shape
        H, Dh = (Wq.shape[1], Wq.shape[2])
        M = mem0.shape[1]
        scale = Dh ** (-0.5)
        n_seg = S // seg_len
        L = M + seg_len
        idx = jnp.arange(L)
        mask = (idx[:, None] < M) | (idx[:, None] >= idx[None, :])
        mem = mem0
        outs = []
        for s in range(n_seg):
            xs = x[:, s * seg_len:(s + 1) * seg_len, :].copy()
            h = jnp.concatenate([mem, xs], axis=1)
            q = jnp.einsum('btd,dhe->bhte', h, Wq)
            k = jnp.einsum('btd,dhe->bhte', h, Wk)
            v = jnp.einsum('btd,dhe->bhte', h, Wv)
            scores = jnp.einsum('bhqe,bhke->bhqk', q, k) * scale
            scores = jnp.where(mask[None, None], scores, -1000000000.0)
            p = _softmax(scores, axis=-1)
            o = jnp.einsum('bhqk,bhke->bhqe', p, v)
            o = jnp.einsum('bhte,hed->btd', o, Wo)
            mem = o[:, :M, :].copy()
            outs.append(o[:, M:, :])
        return jnp.concatenate(outs, axis=1)

    def _B_ref(x, wqkv, wo):
        B, S, D = x.shape
        H = 32
        Dh = D // H
        W, dil = (8, 2)
        qkv = (lambda x, *d: x.transpose(*d))((x @ wqkv).reshape(B, S, 3, H, Dh), 2, 0, 3, 1, 4)
        q, k, v = (qkv[0], qkv[1], qkv[2])
        scale = Dh ** (-0.5)
        pos = jnp.arange(S)
        off = jnp.arange(W) * dil
        idx = pos[:, None] - off[None, :]
        mask = idx >= 0
        idx_c = jnp.where(mask, idx, 0).reshape(-1)
        kg = k[:, :, idx_c, :].reshape(B, H, S, W, Dh)
        vg = v[:, :, idx_c, :].reshape(B, H, S, W, Dh)
        logits = jnp.einsum('bhsd,bhswd->bhsw', q, kg) * scale
        logits = jnp.where(mask[None, None, :, :], logits, -1000000000.0)
        attn = _softmax(logits, axis=-1)
        o = jnp.einsum('bhsw,bhswd->bhsd', attn, vg)
        return (lambda x, *d: x.transpose(*d))(o, 0, 2, 1, 3).reshape(B, S, D) @ wo
    x = A_x
    x = x + _A_ref(_layernorm(x, axis=-1), A_mem0, A_Wq, A_Wk, A_Wv, A_Wo, A_seg_len)
    x = x + _B_ref(_layernorm(x, axis=-1), B_wqkv, B_wo)
    x = x + _A_ref(_layernorm(x, axis=-1), A_mem0, A_Wq, A_Wk, A_Wv, A_Wo, A_seg_len)
    x = x + _B_ref(_layernorm(x, axis=-1), B_wqkv, B_wo)
    return x
```

```python
import functools

import jax
import jax.numpy as jnp
from jax import lax
import jax.experimental.pallas as pl
import jax.experimental.pallas.tpu as pltpu

F32 = jnp.float32
BF16 = jnp.bfloat16
NEG = -1000000000.0

_NN = (((1,), (0,)), ((), ()))
_NT = (((1,), (1,)), ((), ()))


def _dot(a, b, dims=_NN):
    return lax.dot_general(a, b, dims, preferred_element_type=F32)


def _layernorm(x):
    d = x.shape[-1]
    m = jnp.sum(x, axis=-1, keepdims=True) * (1.0 / d)
    xc = x - m
    v = jnp.sum(xc * xc, axis=-1, keepdims=True) * (1.0 / d)
    return xc * lax.rsqrt(v + 1e-05)


def _kernel(x_ref, mem0_ref, wq_ref, wk_ref, wv_ref, wo_ref, bqkv_ref, bwo_ref,
            out_ref, xbuf, h_s, o_s, qb_s, kb_s, vb_s, bq_s, bo_s,
            *, S, D, H, Dh, M, SEG, HB, W, DIL):
    L = M + SEG
    n_seg = S // SEG
    NP = H // 2
    PW = 2 * Dh
    DB = D // HB
    HALO = 16
    scale_a = Dh ** (-0.5)
    scale_b = DB ** (-0.5)

    row = lax.broadcasted_iota(jnp.int32, (L, 128), 0)
    lane = lax.broadcasted_iota(jnp.int32, (L, 128), 1)
    key = jnp.where(lane < L, lane, lane - L)
    in_a = lane < L
    in_b = jnp.logical_and(lane >= L, lane < 2 * L)
    causal = jnp.logical_or(row < M, row >= key)
    mask_ab = jnp.logical_and(causal, lane < 2 * L)
    lo64 = lane < (Dh - 128)

    r_i = lax.broadcasted_iota(jnp.int32, (D, D), 0)
    c_i = lax.broadcasted_iota(jnp.int32, (D, D), 1)
    perm = (r_i == (c_i % HB) * DB + c_i // HB).astype(BF16)
    permT = (c_i == (r_i % HB) * DB + r_i // HB).astype(BF16)
    for t in range(3):
        bq_s[:, t * D:(t + 1) * D] = _dot(bqkv_ref[:, t * D:(t + 1) * D], perm).astype(BF16)
    bo_s[...] = _dot(permT, bwo_ref[...]).astype(BF16)

    xbuf[...] = x_ref[...].astype(F32)
    kb_s[0:HALO, :] = jnp.zeros((HALO, D), F32)
    vb_s[0:HALO, :] = jnp.zeros((HALO, D), F32)

    def a_step(s, mem):
        r0 = pl.multiple_of(s * SEG, SEG)
        xs = xbuf[pl.ds(r0, SEG), :]
        h_s[0:M, :] = mem
        h_s[M:L, :] = _layernorm(xs)
        h = h_s[...]
        for p in range(NP):
            c0 = p * PW
            q = _dot(h, wq_ref[:, c0:c0 + PW])
            k = _dot(h, wk_ref[:, c0:c0 + PW])
            v = _dot(h, wv_ref[:, c0:c0 + PW])
            z = jnp.zeros((L, 128), F32)
            k1, v1 = k[:, 128:256], v[:, 128:256]
            kb = jnp.concatenate([
                jnp.concatenate([k[:, 0:128], jnp.where(lo64, k1, 0.0), z], axis=1),
                jnp.concatenate([z, jnp.where(lo64, 0.0, k1), k[:, 256:384]], axis=1)], axis=0)
            vb = jnp.concatenate([
                jnp.concatenate([v[:, 0:128], jnp.where(lo64, v1, 0.0), z], axis=1),
                jnp.concatenate([z, jnp.where(lo64, 0.0, v1), v[:, 256:384]], axis=1),
                jnp.zeros((128 - 2 * L, PW), F32)], axis=0)
            kb = jnp.concatenate([kb, jnp.zeros((128 - 2 * L, PW), F32)], axis=0)
            sc = _dot(q, kb.astype(BF16), _NT)
            sc = jnp.where(mask_ab, sc * scale_a, NEG)
            ma = jnp.max(jnp.where(in_a, sc, NEG), axis=-1, keepdims=True)
            mb = jnp.max(jnp.where(in_b, sc, NEG), axis=-1, keepdims=True)
            e = jnp.exp(sc - jnp.where(in_a, ma, mb))
            e = jnp.where(mask_ab, e, 0.0)
            la = jnp.sum(jnp.where(in_a, e, 0.0), axis=-1, keepdims=True)
            lb = jnp.sum(jnp.where(in_b, e, 0.0), axis=-1, keepdims=True)
            pr = e * jnp.where(in_a, 1.0 / la, 1.0 / lb)
            o_s[:, c0:c0 + PW] = _dot(pr, vb.astype(BF16))
        o = _dot(o_s[...], wo_ref[...])
        xbuf[pl.ds(r0, SEG), :] = xs + o[M:L, :]
        return o[0:M, :]

    def b_step(s, _):
        r0 = pl.multiple_of(s * SEG, SEG)
        xs = xbuf[pl.ds(r0, SEG), :]
        y = _layernorm(xs)
        qkv = _dot(y, bq_s[...])
        q = qkv[:, 0:D] * scale_b
        kb_s[pl.ds(r0 + HALO, SEG), :] = qkv[:, D:2 * D]
        vb_s[pl.ds(r0 + HALO, SEG), :] = qkv[:, 2 * D:3 * D]
        kw = kb_s[pl.ds(r0, SEG + HALO), :]
        vw = vb_s[pl.ds(r0, SEG + HALO), :]
        pos = r0 + lax.broadcasted_iota(jnp.int32, (SEG, 128), 0)
        lg = []
        for w in range(W):
            o0 = HALO - DIL * w
            pr = q * kw[o0:o0 + SEG, :]
            t = pr[:, 0:128]
            for j in range(1, D // 128):
                t = t + pr[:, j * 128:(j + 1) * 128]
            t = t + pltpu.roll(t, 64, 1)
            t = t + pltpu.roll(t, 32, 1)
            lg.append(jnp.where(pos >= DIL * w, t, NEG))
        mx = lg[0]
        for w in range(1, W):
            mx = jnp.maximum(mx, lg[w])
        es = [jnp.exp(l - mx) for l in lg]
        den = es[0]
        for w in range(1, W):
            den = den + es[w]
        inv = 1.0 / den
        acc = None
        for w in range(W):
            o0 = HALO - DIL * w
            pw = es[w] * inv
            pw5 = jnp.concatenate([pw] * (D // 128), axis=1)
            term = pw5 * vw[o0:o0 + SEG, :]
            acc = term if acc is None else acc + term
        xbuf[pl.ds(r0, SEG), :] = xs + _dot(acc, bo_s[...])
        return 0

    for _layer in range(2):
        lax.fori_loop(0, n_seg, a_step, mem0_ref[...].astype(F32))
        lax.fori_loop(0, n_seg, b_step, 0)
    out_ref[...] = xbuf[...].astype(out_ref.dtype)


@jax.jit
def pallas_interleave_layers__memory_aug_recurrent_mem_tr__sliding_local_dilated__prompt_kernel(
    A_x: jax.Array,
    A_mem0: jax.Array,
    A_Wq: jax.Array,
    A_Wk: jax.Array,
    A_Wv: jax.Array,
    A_Wo: jax.Array,
    A_seg_len,
    B_x: jax.Array,
    B_wqkv: jax.Array,
    B_wo: jax.Array,
):
    del B_x
    B, S, D = A_x.shape
    _, H, Dh = A_Wq.shape
    M = A_mem0.shape[1]
    SEG = 32
    HB, W, DIL = 32, 8, 2
    L = M + SEG
    kern = functools.partial(_kernel, S=S, D=D, H=H, Dh=Dh, M=M, SEG=SEG, HB=HB, W=W, DIL=DIL)
    out = pl.pallas_call(
        kern,
        out_shape=jax.ShapeDtypeStruct((S, D), A_x.dtype),
        scratch_shapes=[
            pltpu.VMEM((S, D), F32),
            pltpu.VMEM((L, D), F32),
            pltpu.VMEM((L, H * Dh), F32),
            pltpu.VMEM((8, 128), F32),
            pltpu.VMEM((S + 16, D), F32),
            pltpu.VMEM((S + 16, D), F32),
            pltpu.VMEM((D, 3 * D), BF16),
            pltpu.VMEM((D, D), BF16),
        ],
        compiler_params=pltpu.CompilerParams(vmem_limit_bytes=110 * 2**20),
        name="rmt_sliding",
    )(
        A_x.reshape(S, D), A_mem0.reshape(M, D),
        A_Wq.reshape(D, H * Dh), A_Wk.reshape(D, H * Dh), A_Wv.reshape(D, H * Dh),
        A_Wo.reshape(H * Dh, D), B_wqkv, B_wo,
    )
    return out.reshape(B, S, D)
```

```python
import functools

import jax
import jax.numpy as jnp
from jax import lax
import jax.experimental.pallas as pl
import jax.experimental.pallas.tpu as pltpu

F32 = jnp.float32
BF16 = jnp.bfloat16
NEG = -1000000000.0
LOG2E = 1.4426950408889634

_NN = (((1,), (0,)), ((), ()))
_NT = (((1,), (1,)), ((), ()))


def _dot(a, b, dims=_NN):
    return lax.dot_general(a, b, dims, preferred_element_type=F32)


def _as_bf16(u):
    return pltpu.bitcast(u, BF16)


def _as_u32(b):
    return pltpu.bitcast(b, jnp.uint32)


def _layernorm(x):
    d = x.shape[-1]
    m = jnp.sum(x, axis=-1, keepdims=True) * (1.0 / d)
    xc = x - m
    v = jnp.sum(xc * xc, axis=-1, keepdims=True) * (1.0 / d)
    return xc * lax.rsqrt(v + 1e-05)


def _make_schedule(NP):
    sched = []
    hold = (NP - 4, NP - 3)
    nxt_o = 0
    for i in range(NP):
        if i in hold:
            sched += [("Pk", i), ("Pq", i), ("Pv", i), ("V", i - 1), ("S", i)]
            continue
        sched += [("Pk", i), ("Pq", i)]
        if i == 1:
            sched.append(("Bqkv", 0))
        if i >= 2:
            sched.append(("O", nxt_o))
            nxt_o += 1
        if i >= 1:
            sched.append(("V", i - 1))
        sched += [("Pv", i), ("S", i)]
    while nxt_o < NP - 1:
        sched.append(("O", nxt_o))
        nxt_o += 1
    sched += [("V", NP - 1), ("Bo", 0), ("O", NP - 1)]
    return sched


def _kernel(x_ref, mem0_ref, wqt_hbm, wkt_hbm, wvt_hbm, wo_hbm, bqkv_ref, bwo_ref,
            out_ref, xbuf, xn_a, xn_b, kb_s, vb_s, bq_s, bo_s, stage, w_s, wo_s, sems,
            *, S, D, H, Dh, M, SEG, HB, W, DIL):
    L = M + SEG
    n_seg = S // SEG
    NP = H // 2
    PW = 2 * Dh
    HD = H * Dh
    DB = D // HB
    HALO = 16
    PAD = SEG
    scale_a = Dh ** (-0.5)
    scale_b = DB ** (-0.5)
    CH = 512
    NCH = HD // CH

    def wcopy(t, c):
        src = (wqt_hbm, wkt_hbm, wvt_hbm, wo_hbm)[t]
        return pltpu.make_async_copy(src.at[pl.ds(c * CH, CH), :], stage.at[t, pl.ds(c * CH, CH), :], sems.at[t, c])

    for c in range(NCH):
        for t in range(3):
            wcopy(t, c).start()
    for c in range(NCH):
        wcopy(3, c).start()

    row = lax.broadcasted_iota(jnp.int32, (L, 128), 0)
    lane = lax.broadcasted_iota(jnp.int32, (L, 128), 1)
    key = jnp.where(lane < L, lane, lane - L)
    in_a = lane < L
    in_b = jnp.logical_and(lane >= L, lane < 2 * L)
    causal = jnp.logical_or(row < M, row >= key)
    mask_ab = jnp.logical_and(causal, lane < 2 * L)
    lo64 = lane < (Dh - 128)

    r_i = lax.broadcasted_iota(jnp.int32, (D, D), 0)
    c_i = lax.broadcasted_iota(jnp.int32, (D, D), 1)
    perm = (r_i == (c_i % HB) * DB + c_i // HB).astype(BF16)
    permT = (c_i == (r_i % HB) * DB + r_i // HB).astype(BF16)
    for t in range(3):
        bq_s[:, t * D:(t + 1) * D] = _as_u32(_dot(bqkv_ref[:, t * D:(t + 1) * D], perm).astype(BF16))
    bo_s[...] = _as_u32(_dot(permT, bwo_ref[...]).astype(BF16))

    kb_s[0:HALO, :] = jnp.zeros((HALO, D), F32)
    vb_s[0:HALO, :] = jnp.zeros((HALO, D), F32)
    xbuf[0:PAD, :] = jnp.zeros((PAD, D), F32)

    def ln0(i, _):
        r0 = pl.multiple_of(i * 64, 64)
        xs = x_ref[pl.ds(r0, 64), :].astype(F32)
        xbuf[pl.ds(PAD + r0, 64), :] = xs
        xn_a[pl.ds(r0, 64), :] = _layernorm(xs)
        return 0
    lax.fori_loop(0, S // 64, ln0, 0)

    for c in range(NCH):
        for t in range(3):
            wcopy(t, c).wait()
            wt = stage[t, c * CH:(c + 1) * CH, :].T
            for j in range(CH // 128):
                n = c * (CH // 128) + j
                p, r = divmod(n, 3)
                w_s[:, (p * 9 + t * 3 + r) * 128:(p * 9 + t * 3 + r + 1) * 128] = _as_u32(wt[:, j * 128:(j + 1) * 128])
    for c in range(NCH):
        wcopy(3, c).wait()
        wo_s[c * CH // 2:(c + 1) * CH // 2, :] = _as_u32(stage[3, c * CH:(c + 1) * CH, :])

    def b_ln(sb):
        r0 = pl.multiple_of((sb + 1) * SEG, SEG)
        xs = xbuf[pl.ds(r0, SEG), :]
        return xs, _layernorm(xs)

    def b_qkv(sb, y):
        r0 = pl.multiple_of((sb + 1) * SEG, SEG)
        qkv = _dot(y, _as_bf16(bq_s[...]))
        q = qkv[:, 0:D] * (scale_b * LOG2E)
        kb_s[pl.ds(r0 + HALO, SEG), :] = qkv[:, D:2 * D]
        vb_s[pl.ds(r0 + HALO, SEG), :] = qkv[:, 2 * D:3 * D]
        kw = kb_s[pl.ds(r0, SEG + HALO), :]
        vw = vb_s[pl.ds(r0, SEG + HALO), :]
        pos = sb * SEG + lax.broadcasted_iota(jnp.int32, (SEG, 128), 0)
        lg = []
        for w in range(W):
            o0 = HALO - DIL * w
            pr = q * kw[o0:o0 + SEG, :]
            t = pr[:, 0:128]
            for j in range(1, D // 128):
                t = t + pr[:, j * 128:(j + 1) * 128]
            t = t + pltpu.roll(t, 64, 1)
            t = t + pltpu.roll(t, 32, 1)
            lg.append(jnp.where(pos >= DIL * w, t, NEG * LOG2E))
        mx = lg[0]
        for w in range(1, W):
            mx = jnp.maximum(mx, lg[w])
        es = [jnp.exp2(l - mx) for l in lg]
        den = es[0]
        for w in range(1, W):
            den = den + es[w]
        inv = 1.0 / den
        acc = None
        for w in range(W):
            o0 = HALO - DIL * w
            pw = es[w] * inv
            pw5 = jnp.concatenate([pw] * (D // 128), axis=1)
            term = pw5 * vw[o0:o0 + SEG, :]
            acc = term if acc is None else acc + term
        return acc

    def b_out(sb, xs, acc, last):
        x2 = xs + _dot(acc, _as_bf16(bo_s[...]))
        if last:
            out_ref[pl.ds(pl.multiple_of(jnp.maximum(sb, 0) * SEG, SEG), SEG), :] = x2.astype(out_ref.dtype)
        else:
            xbuf[pl.ds(pl.multiple_of((sb + 1) * SEG, SEG), SEG), :] = x2
            xn_b[pl.ds(pl.multiple_of((sb + 1) * SEG, SEG), SEG), :] = _layernorm(x2)

    sched = _make_schedule(NP)

    def make_step(xn_in, last):
        def step(s, mem):
            r0 = pl.multiple_of(s * SEG, SEG)
            xn_off = 0 if xn_in is xn_a else PAD
            h = jnp.concatenate([mem, xn_in[pl.ds(r0 + xn_off, SEG), :]], axis=0)
            bx, by = b_ln(s - 1)
            kb, vb, qq, pr, oo = {}, {}, {}, {}, {}
            out = None
            bacc = None
            z = jnp.zeros((L, 128), F32)

            def blockdiag(a):
                a1 = a[:, 128:256]
                return jnp.concatenate([
                    jnp.concatenate([a[:, 0:128], jnp.where(lo64, a1, 0.0), z], axis=1),
                    jnp.concatenate([z, jnp.where(lo64, 0.0, a1), a[:, 256:384]], axis=1),
                    jnp.zeros((128 - 2 * L, PW), F32)], axis=0).astype(BF16)

            for op, p in sched:
                c0 = p * 9 * 128
                if op == "Pq":
                    qq[p] = _dot(h, _as_bf16(w_s[:, c0:c0 + PW]))
                elif op == "Pk":
                    kb[p] = blockdiag(_dot(h, _as_bf16(w_s[:, c0 + PW:c0 + 2 * PW])))
                elif op == "Pv":
                    vb[p] = blockdiag(_dot(h, _as_bf16(w_s[:, c0 + 2 * PW:c0 + 3 * PW])))
                elif op == "S":
                    sc = _dot(qq.pop(p), kb.pop(p), _NT)
                    sc = jnp.where(mask_ab, sc * (scale_a * LOG2E), NEG * LOG2E)
                    ma = jnp.max(jnp.where(in_a, sc, NEG * LOG2E), axis=-1, keepdims=True)
                    mb = jnp.max(jnp.where(in_b, sc, NEG * LOG2E), axis=-1, keepdims=True)
                    e = jnp.exp2(sc - jnp.where(in_a, ma, mb))
                    la = jnp.sum(jnp.where(in_a, e, 0.0), axis=-1, keepdims=True)
                    lb = jnp.sum(jnp.where(in_b, e, 0.0), axis=-1, keepdims=True)
                    pr[p] = e * (1.0 / jnp.where(in_a, la, lb))
                elif op == "V":
                    oo[p] = _dot(pr.pop(p), vb.pop(p))
                elif op == "O":
                    t = _dot(oo.pop(p), _as_bf16(wo_s[p * PW // 2:(p + 1) * PW // 2, :]))
                    out = t if out is None else out + t
                elif op == "Bqkv":
                    bacc = b_qkv(s - 1, by)
                elif op == "Bo":
                    b_out(s - 1, bx, bacc, last)
            xbuf[pl.ds(r0 + PAD, SEG), :] = xbuf[pl.ds(r0 + PAD, SEG), :] + out[M:L, :]
            return out[0:M, :]
        return step

    for layer in range(2):
        last = layer == 1
        lax.fori_loop(0, n_seg, make_step(xn_a if layer == 0 else xn_b, last), mem0_ref[...].astype(F32))
        bx, by = b_ln(n_seg - 1)
        b_out(n_seg - 1, bx, b_qkv(n_seg - 1, by), last)


@functools.partial(jax.jit, static_argnames=("A_seg_len",))
def pallas_interleave_layers__memory_aug_recurrent_mem_tr__sliding_local_dilated__prompt_kernel(
    A_x: jax.Array,
    A_mem0: jax.Array,
    A_Wq: jax.Array,
    A_Wk: jax.Array,
    A_Wv: jax.Array,
    A_Wo: jax.Array,
    A_seg_len,
    B_x: jax.Array,
    B_wqkv: jax.Array,
    B_wo: jax.Array,
):
    del B_x
    B, S, D = A_x.shape
    _, H, Dh = A_Wq.shape
    M = A_mem0.shape[1]
    SEG = int(A_seg_len)
    HB, W, DIL = 32, 8, 2
    L = M + SEG
    HD = H * Dh
    kern = functools.partial(_kernel, S=S, D=D, H=H, Dh=Dh, M=M, SEG=SEG, HB=HB, W=W, DIL=DIL)
    tr = lambda w: jnp.transpose(w, (1, 2, 0)).reshape(HD, D)
    hbm = pl.BlockSpec(memory_space=pl.ANY)
    vm = pl.BlockSpec(memory_space=pltpu.VMEM)
    out = pl.pallas_call(
        kern,
        out_shape=jax.ShapeDtypeStruct((S, D), A_x.dtype),
        in_specs=[vm, vm, hbm, hbm, hbm, hbm, vm, vm],
        out_specs=vm,
        scratch_shapes=[
            pltpu.VMEM((S + SEG, D), F32),
            pltpu.VMEM((S, D), F32),
            pltpu.VMEM((S + SEG, D), F32),
            pltpu.VMEM((S + SEG + 16, D), F32),
            pltpu.VMEM((S + SEG + 16, D), F32),
            pltpu.VMEM((D // 2, 3 * D), jnp.uint32),
            pltpu.VMEM((D // 2, D), jnp.uint32),
            pltpu.VMEM((4, HD, D), BF16),
            pltpu.VMEM((D // 2, 3 * HD), jnp.uint32),
            pltpu.VMEM((HD // 2, D), jnp.uint32),
            pltpu.SemaphoreType.DMA((4, HD // 512)),
        ],
        compiler_params=pltpu.CompilerParams(vmem_limit_bytes=120 * 2**20),
        name="rmt_sliding",
    )(
        A_x.reshape(S, D), A_mem0.reshape(M, D),
        tr(A_Wq), tr(A_Wk), tr(A_Wv),
        A_Wo.reshape(HD, D), B_wqkv, B_wo,
    )
    return out.reshape(B, S, D)
```

```python
import functools

import jax
import jax.numpy as jnp
from jax import lax
import jax.experimental.pallas as pl
import jax.experimental.pallas.tpu as pltpu

F32 = jnp.float32
BF16 = jnp.bfloat16
NEG = -1000000000.0
LOW = -3.0e38
LOG2E = 1.4426950408889634

_NN = (((1,), (0,)), ((), ()))
_NT = (((1,), (1,)), ((), ()))


def _dot(a, b, dims=_NN):
    return lax.dot_general(a, b, dims, preferred_element_type=F32)


def _as_bf16(u):
    return pltpu.bitcast(u, BF16)


def _as_u32(b):
    return pltpu.bitcast(b, jnp.uint32)


def _layernorm(x):
    d = x.shape[-1]
    m = jnp.sum(x, axis=-1, keepdims=True) * (1.0 / d)
    xc = x - m
    v = jnp.sum(xc * xc, axis=-1, keepdims=True) * (1.0 / d)
    return xc * lax.rsqrt(v + 1e-05)


def _make_schedule(NP):
    sched = []
    bo_slot = NP - 5
    hold = (NP - 4, NP - 3)
    nxt_o = 0
    for i in range(NP):
        sched += [("Pk", i)]
        if i == 0 or 2 <= i < bo_slot or i == bo_slot + 2:
            sched.append(("B", i))
        sched += [("Pq", i)]
        if i == 1 or i == bo_slot:
            sched.append(("B", i))
        elif i >= 2 and i not in hold:
            sched.append(("O", nxt_o))
            nxt_o += 1
        sched.append(("Pv", i))
        if i >= 1:
            sched.append(("V", i - 1))
        sched.append(("S", i))
    while nxt_o < NP - 2:
        sched.append(("O", nxt_o))
        nxt_o += 1
    sched += [("V", NP - 1), ("O", NP - 2), ("O", NP - 1)]
    return sched


def _finish(gen):
    for _ in gen:
        pass


def _kernel(x_hbm, mem0_hbm, wqt_hbm, wkt_hbm, wvt_hbm, wo_hbm, bqkv_hbm, bwo_hbm,
            out_hbm, xbuf, xn_a, xn_b, qb_s, kb_s, vb_s, bq_s, bo_s, stage, w_s, wo_s,
            xio, bq_st, bo_st, mem_st, sems, sem_b, sem_o,
            *, S, D, H, Dh, M, SEG, HB, W, DIL):
    L = M + SEG
    n_seg = S // SEG
    NP = H // 2
    PW = 2 * Dh
    HD = H * Dh
    DB = D // HB
    HALO = 16
    PAD = SEG
    JUNK = S + SEG + HALO
    scale_a = Dh ** (-0.5)
    scale_b = DB ** (-0.5)
    CH = 512
    NCH = HD // CH
    XCH = 512
    NXC = S // XCH

    def wcopy(t, c):
        src = (wqt_hbm, wkt_hbm, wvt_hbm, wo_hbm)[t]
        return pltpu.make_async_copy(src.at[pl.ds(c * CH, CH), :], stage.at[t, pl.ds(c * CH, CH), :], sems.at[t, c])

    def xcopy(c):
        return pltpu.make_async_copy(x_hbm.at[pl.ds(c * XCH, XCH), :], xio.at[pl.ds(c * XCH, XCH), :], sem_b.at[4 + c])

    def bcopy(t):
        if t < 3:
            return pltpu.make_async_copy(bqkv_hbm.at[:, pl.ds(t * D, D)], bq_st.at[:, pl.ds(t * D, D)], sem_b.at[t])
        return pltpu.make_async_copy(bwo_hbm, bo_st, sem_b.at[3])

    queue = ([xcopy(c) for c in range(NXC)] + [bcopy(t) for t in range(4)]
             + [wcopy(3, c) for c in range(NCH)]
             + [wcopy(t, c) for c in range(NCH) for t in range(3)])
    queue.reverse()

    def start_next(n):
        for _ in range(n):
            if queue:
                queue.pop().start()

    mem_copy = pltpu.make_async_copy(mem0_hbm, mem_st.at[pl.ds(0, M), :], sem_b.at[4 + NXC])
    mem_copy.start()
    start_next(4)

    row = lax.broadcasted_iota(jnp.int32, (L, 128), 0)
    lane = lax.broadcasted_iota(jnp.int32, (L, 128), 1)
    key = jnp.where(lane < L, lane, lane - L)
    in_a = lane < L
    in_b = jnp.logical_and(lane >= L, lane < 2 * L)
    causal = jnp.logical_or(row < M, row >= key)
    mask_ab = jnp.logical_and(causal, lane < 2 * L)
    fill_a = jnp.where(lane < 2 * L, NEG * LOG2E, LOW)
    lo64 = lane < (Dh - 128)

    kb_s[0:HALO, :] = jnp.zeros((HALO, D), F32)
    vb_s[0:HALO, :] = jnp.zeros((HALO, D), F32)
    xbuf[0:PAD, :] = jnp.zeros((PAD, D), F32)

    for c in range(NXC):
        xcopy(c).wait()
        start_next(1)

        def ln0(i, _):
            r0 = pl.multiple_of(c * XCH + i * 128, 128)
            xs = xio[pl.ds(r0, 128), :].astype(F32)
            xbuf[pl.ds(PAD + r0, 128), :] = xs
            xn_a[pl.ds(r0, 128), :] = _layernorm(xs)
            return 0
        lax.fori_loop(0, XCH // 128, ln0, 0)

    r_i = lax.broadcasted_iota(jnp.int32, (D, D), 0)
    c_i = lax.broadcasted_iota(jnp.int32, (D, D), 1)
    perm = (r_i == (c_i % HB) * DB + c_i // HB).astype(BF16)
    permT = (c_i == (r_i % HB) * DB + r_i // HB).astype(BF16)
    for t in range(3):
        bcopy(t).wait()
        start_next(3)
        bq_s[:, t * D:(t + 1) * D] = _as_u32(_dot(bq_st[:, t * D:(t + 1) * D], perm).astype(BF16))
    bcopy(3).wait()
    start_next(3)
    bo_s[...] = _as_u32(_dot(permT, bo_st[...]).astype(BF16))

    for c in range(NCH):
        wcopy(3, c).wait()
        start_next(1 if c >= 6 else 0)
        wo_s[c * CH // 2:(c + 1) * CH // 2, :] = _as_u32(stage[3, c * CH:(c + 1) * CH, :])
    for c in range(NCH):
        for t in range(3):
            wcopy(t, c).wait()
            start_next(1)
            wt = stage[t, c * CH:(c + 1) * CH, :].T
            for j in range(CH // 128):
                n = c * (CH // 128) + j
                p, r = divmod(n, 3)
                w_s[:, (p * 9 + t * 3 + r) * 128:(p * 9 + t * 3 + r + 1) * 128] = _as_u32(wt[:, j * 128:(j + 1) * 128])

    def b_stages(sb, last):
        r0 = pl.multiple_of((sb + 1) * SEG, SEG)
        tok = yield
        if tok is not None and GATE_LN:
            xbuf[JUNK:JUNK + 8, 0:128] = tok
        y = _layernorm(xbuf[pl.ds(r0, SEG), :])
        tok = yield
        qkv = _dot(y, _as_bf16(bq_s[...]))
        qb_s[...] = qkv[:, 0:D]
        kb_s[pl.ds(r0 + HALO, SEG), :] = qkv[:, D:2 * D]
        vb_s[pl.ds(r0 + HALO, SEG), :] = qkv[:, 2 * D:3 * D]
        pos = sb * SEG + lax.broadcasted_iota(jnp.int32, (SEG, 128), 0)
        lg = [None] * W
        for j in range(W // 2):
            tok = yield
            if tok is not None:
                kb_s[JUNK:JUNK + 8, 0:128] = tok
            kw = kb_s[pl.ds(r0, SEG + HALO), :]
            q = qb_s[...]
            o0 = HALO - DIL * (j + W // 2)
            kj = kw[o0:o0 + SEG + 8, :]
            for w, ko in ((j, 8), (j + W // 2, 0)):
                pr = q * kj[ko:ko + SEG, :]
                t = pr[:, 0:128]
                for c in range(1, D // 128):
                    t = t + pr[:, c * 128:(c + 1) * 128]
                t = t + pltpu.roll(t, 64, 1)
                t = t + pltpu.roll(t, 32, 1)
                lg[w] = jnp.where(pos >= DIL * w, t * (scale_b * LOG2E), NEG * LOG2E)
        tok = yield
        mx = lg[0]
        for w in range(1, W):
            mx = jnp.maximum(mx, lg[w])
        es = [jnp.exp2(l - mx) for l in lg]
        den = es[0]
        for w in range(1, W):
            den = den + es[w]
        inv = 1.0 / den
        ps = [e * inv for e in es]
        acc = None
        for j in range(W // 2):
            tok = yield
            if tok is not None:
                vb_s[JUNK:JUNK + 8, 0:128] = tok
            vw = vb_s[pl.ds(r0, SEG + HALO), :]
            o0 = HALO - DIL * (j + W // 2)
            vj = vw[o0:o0 + SEG + 8, :]
            for w, ko in ((j, 8), (j + W // 2, 0)):
                pw5 = jnp.concatenate([ps[w]] * (D // 128), axis=1)
                term = pw5 * vj[ko:ko + SEG, :]
                acc = term if acc is None else acc + term
        tok = yield
        x2 = xbuf[pl.ds(r0, SEG), :] + _dot(acc, _as_bf16(bo_s[...]))
        if last:
            xio[pl.ds(pl.multiple_of(jnp.maximum(sb, 0) * SEG, SEG), SEG), :] = x2.astype(xio.dtype)
        else:
            xbuf[pl.ds(r0, SEG), :] = x2
            tok = yield
            if tok is not None and GATE_LN:
                xbuf[JUNK:JUNK + 8, 0:128] = tok
            xn_b[pl.ds(r0, SEG), :] = _layernorm(xbuf[pl.ds(r0, SEG), :])

    GATE_LN = True
    sched = _make_schedule(NP)
    z = jnp.zeros((L, 128), F32)

    def blockdiag(a):
        a1 = a[:, 128:256]
        return jnp.concatenate([
            jnp.concatenate([a[:, 0:128], jnp.where(lo64, a1, 0.0), z], axis=1),
            jnp.concatenate([z, jnp.where(lo64, 0.0, a1), a[:, 256:384]], axis=1),
            jnp.zeros((128 - 2 * L, PW), F32)], axis=0).astype(BF16)

    def advance(gen, token):
        try:
            gen.send(token)
        except StopIteration:
            pass

    def make_step(xn_in, last):
        def step(s, mem):
            r0 = pl.multiple_of(s * SEG, SEG)
            xn_off = 0 if xn_in is xn_a else PAD
            h = jnp.concatenate([mem, xn_in[pl.ds(r0 + xn_off, SEG), :]], axis=0)
            bgen = b_stages(s - 1, last)
            next(bgen)
            kb, vb, qq, pr, oo = {}, {}, {}, {}, {}
            out = None
            token = None
            for op, p in sched:
                c0 = p * 9 * 128
                if op == "Pq":
                    qq[p] = _dot(h, _as_bf16(w_s[:, c0:c0 + PW]))
                elif op == "Pk":
                    kk = _dot(h, _as_bf16(w_s[:, c0 + PW:c0 + 2 * PW]))
                    token = kk[0:8, 0:128]
                    kb[p] = blockdiag(kk)
                elif op == "Pv":
                    vb[p] = blockdiag(_dot(h, _as_bf16(w_s[:, c0 + 2 * PW:c0 + 3 * PW])))
                elif op == "S":
                    sc = _dot(qq.pop(p), kb.pop(p), _NT)
                    sc = jnp.where(mask_ab, sc * (scale_a * LOG2E), fill_a)
                    ma = jnp.max(jnp.where(in_a, sc, LOW), axis=-1, keepdims=True)
                    mb = jnp.max(jnp.where(in_b, sc, LOW), axis=-1, keepdims=True)
                    e = jnp.exp2(sc - jnp.where(in_a, ma, mb))
                    la = jnp.sum(jnp.where(in_a, e, 0.0), axis=-1, keepdims=True)
                    lb = jnp.sum(jnp.where(in_b, e, 0.0), axis=-1, keepdims=True)
                    pr[p] = e * (1.0 / jnp.where(in_a, la, lb))
                elif op == "V":
                    oo[p] = _dot(pr.pop(p), vb.pop(p))
                elif op == "O":
                    t = _dot(oo.pop(p), _as_bf16(wo_s[p * PW // 2:(p + 1) * PW // 2, :]))
                    out = t if out is None else out + t
                elif op == "B":
                    advance(bgen, token)
            _finish(bgen)
            xbuf[pl.ds(r0 + PAD, SEG), :] = xbuf[pl.ds(r0 + PAD, SEG), :] + out[M:L, :]
            return out[0:M, :]
        return step

    def ocopy(c):
        return pltpu.make_async_copy(xio.at[pl.ds(c * XCH, XCH), :], out_hbm.at[pl.ds(c * XCH, XCH), :], sem_o.at[c])

    mem_copy.wait()
    mem0 = mem_st[0:M, :].astype(F32)
    lax.fori_loop(0, n_seg, make_step(xn_a, False), mem0)
    for _ in b_stages(n_seg - 1, False):
        pass
    SPC = XCH // SEG
    step2 = make_step(xn_b, True)

    def chunk(c, mem):
        mem = lax.fori_loop(c * SPC, (c + 1) * SPC, step2, mem)

        @pl.when(c > 0)
        def _():
            ocopy(c - 1).start()
        return mem
    lax.fori_loop(0, NXC, chunk, mem0)
    for _ in b_stages(n_seg - 1, True):
        pass
    ocopy(NXC - 1).start()
    for c in range(NXC):
        ocopy(c).wait()


@functools.partial(jax.jit, static_argnames=("A_seg_len",))
def pallas_interleave_layers__memory_aug_recurrent_mem_tr__sliding_local_dilated__prompt_kernel(
    A_x: jax.Array,
    A_mem0: jax.Array,
    A_Wq: jax.Array,
    A_Wk: jax.Array,
    A_Wv: jax.Array,
    A_Wo: jax.Array,
    A_seg_len,
    B_x: jax.Array,
    B_wqkv: jax.Array,
    B_wo: jax.Array,
):
    del B_x
    B, S, D = A_x.shape
    _, H, Dh = A_Wq.shape
    M = A_mem0.shape[1]
    SEG = int(A_seg_len)
    HB, W, DIL = 32, 8, 2
    HD = H * Dh
    kern = functools.partial(_kernel, S=S, D=D, H=H, Dh=Dh, M=M, SEG=SEG, HB=HB, W=W, DIL=DIL)
    tr = lambda w: jnp.transpose(w, (1, 2, 0)).reshape(HD, D)
    hbm = pl.BlockSpec(memory_space=pl.ANY)
    vm = pl.BlockSpec(memory_space=pltpu.VMEM)
    out = pl.pallas_call(
        kern,
        out_shape=jax.ShapeDtypeStruct((S, D), A_x.dtype),
        in_specs=[hbm, hbm, hbm, hbm, hbm, hbm, hbm, hbm],
        out_specs=hbm,
        scratch_shapes=[
            pltpu.VMEM((S + SEG + 32, D), F32),
            pltpu.VMEM((S, D), F32),
            pltpu.VMEM((S + SEG, D), F32),
            pltpu.VMEM((SEG, D), F32),
            pltpu.VMEM((S + SEG + 32, D), F32),
            pltpu.VMEM((S + SEG + 32, D), F32),
            pltpu.VMEM((D // 2, 3 * D), jnp.uint32),
            pltpu.VMEM((D // 2, D), jnp.uint32),
            pltpu.VMEM((4, HD, D), BF16),
            pltpu.VMEM((D // 2, 3 * HD), jnp.uint32),
            pltpu.VMEM((HD // 2, D), jnp.uint32),
            pltpu.VMEM((S, D), A_x.dtype),
            pltpu.VMEM((D, 3 * D), BF16),
            pltpu.VMEM((D, D), BF16),
            pltpu.VMEM((64, D), BF16),
            pltpu.SemaphoreType.DMA((4, HD // 512)),
            pltpu.SemaphoreType.DMA((5 + S // 512,)),
            pltpu.SemaphoreType.DMA((S // 512,)),
        ],
        compiler_params=pltpu.CompilerParams(vmem_limit_bytes=120 * 2**20),
        name="rmt_sliding",
    )(
        A_x.reshape(S, D), A_mem0.reshape(M, D),
        tr(A_Wq), tr(A_Wk), tr(A_Wv),
        A_Wo.reshape(HD, D), B_wqkv, B_wo,
    )
    return out.reshape(B, S, D)
```

```python
import functools

import jax
import jax.numpy as jnp
from jax import lax
import jax.experimental.pallas as pl
import jax.experimental.pallas.tpu as pltpu

F32 = jnp.float32
BF16 = jnp.bfloat16
NEG = -1000000000.0
LOW = -3.0e38
LOG2E = 1.4426950408889634

_NN = (((1,), (0,)), ((), ()))
_NT = (((1,), (1,)), ((), ()))


def _dot(a, b, dims=_NN):
    return lax.dot_general(a, b, dims, preferred_element_type=F32)


def _as_bf16(u):
    return pltpu.bitcast(u, BF16)


def _as_u32(b):
    return pltpu.bitcast(b, jnp.uint32)


def _layernorm(x):
    d = x.shape[-1]
    m = jnp.sum(x, axis=-1, keepdims=True) * (1.0 / d)
    xc = x - m
    v = jnp.sum(xc * xc, axis=-1, keepdims=True) * (1.0 / d)
    return xc * lax.rsqrt(v + 1e-05)


def _make_schedule(NP):
    sched = []
    bo_slot = NP - 5
    hold = (NP - 4, NP - 3)
    nxt_o = 0
    for i in range(NP):
        sched.append(("Pk", i))
        if i == 0 or 2 <= i < bo_slot:
            sched.append(("B", i))
        elif i == bo_slot + 2:
            sched.append(("LN", i))
        sched.append(("Pq", i))
        if i == 1 or i == bo_slot:
            sched.append(("B", i))
        elif i >= 2 and i not in hold:
            sched.append(("O", nxt_o))
            nxt_o += 1
        sched.append(("Pv", i))
        if i >= 1:
            sched.append(("V", i - 1))
        sched.append(("S", i))
    while nxt_o < NP - 2:
        sched.append(("O", nxt_o))
        nxt_o += 1
    sched += [("V", NP - 1), ("O", NP - 2), ("O", NP - 1)]
    return sched


def _finish(gen):
    for _ in gen:
        pass


def _advance(gen, token):
    try:
        gen.send(token)
    except StopIteration:
        pass


def _kernel(x_hbm, mem0_hbm, wqt_hbm, wkt_hbm, wvt_hbm, wo_hbm, bqkv_hbm, bwo_hbm,
            out_hbm, xbuf, xn_s, qb_s, kb_s, vb_s, bq_s, bo_s, stage, w_s, wo_s,
            xio, bq_st, bo_st, mem_st, sems, sem_b, sem_o,
            *, S, D, H, Dh, M, SEG, HB, W, DIL):
    L = M + SEG
    n_seg = S // SEG
    NP = H // 2
    PW = 2 * Dh
    DB = D // HB
    HALO = 16
    JUNK = S + HALO
    scale_a = Dh ** (-0.5)
    scale_b = DB ** (-0.5)
    XCH = 512
    NXC = S // XCH

    def wcopy(t, p):
        src = (wqt_hbm, wkt_hbm, wvt_hbm, wo_hbm)[t]
        return pltpu.make_async_copy(src.at[pl.ds(p * PW, PW), :], stage.at[t, pl.ds(p * PW, PW), :], sems.at[t, p])

    def xcopy(c):
        return pltpu.make_async_copy(x_hbm.at[pl.ds(c * XCH, XCH), :], xio.at[pl.ds(c * XCH, XCH), :], sem_b.at[5 + c])

    def bcopy(t):
        if t < 3:
            return pltpu.make_async_copy(bqkv_hbm.at[:, pl.ds(t * D, D)], bq_st.at[:, pl.ds(t * D, D)], sem_b.at[t])
        return pltpu.make_async_copy(bwo_hbm, bo_st, sem_b.at[3])

    mem_copy = pltpu.make_async_copy(mem0_hbm, mem_st.at[pl.ds(0, M), :], sem_b.at[4])

    queue = ([xcopy(0), mem_copy] + [bcopy(t) for t in range(4)]
             + [wcopy(t, p) for p in range(NP) for t in (1, 0, 2, 3)]
             + [xcopy(c) for c in range(1, NXC)])
    queue.reverse()

    def start_next(n):
        for _ in range(n):
            if queue:
                queue.pop().start()

    start_next(6)

    row = lax.broadcasted_iota(jnp.int32, (L, 128), 0)
    lane = lax.broadcasted_iota(jnp.int32, (L, 128), 1)
    key = jnp.where(lane < L, lane, lane - L)
    in_a = lane < L
    in_b = jnp.logical_and(lane >= L, lane < 2 * L)
    causal = jnp.logical_or(row < M, row >= key)
    mask_ab = jnp.logical_and(causal, lane < 2 * L)
    fill_a = jnp.where(lane < 2 * L, NEG * LOG2E, LOW)
    lo64 = lane < (Dh - 128)

    kb_s[0:HALO, :] = jnp.zeros((HALO, D), F32)
    vb_s[0:HALO, :] = jnp.zeros((HALO, D), F32)

    def to_f32(c):
        xcopy(c).wait()
        for i in range(XCH // 128):
            r = c * XCH + i * 128
            xbuf[r:r + 128, :] = xio[r:r + 128, :].astype(F32)

    to_f32(0)
    start_next(2)
    xn_s[0:SEG, :] = _layernorm(xbuf[0:SEG, :])

    r_i = lax.broadcasted_iota(jnp.int32, (D, D), 0)
    c_i = lax.broadcasted_iota(jnp.int32, (D, D), 1)
    perm = (r_i == (c_i % HB) * DB + c_i // HB).astype(BF16)
    permT = (c_i == (r_i % HB) * DB + r_i // HB).astype(BF16)
    for t in range(3):
        bcopy(t).wait()
        start_next(3 if t == 0 else 4)
        bq_s[:, t * D:(t + 1) * D] = _as_u32(_dot(bq_st[:, t * D:(t + 1) * D], perm).astype(BF16))
    bcopy(3).wait()
    start_next(4)
    bo_s[...] = _as_u32(_dot(permT, bo_st[...]).astype(BF16))

    def load_qkv_weights(p):
        for t in (1, 0, 2):
            wcopy(t, p).wait()
            start_next(1)
            wt = stage[t, p * PW:(p + 1) * PW, :].T
            for j in range(PW // 128):
                c = (p * 9 + t * 3 + j) * 128
                w_s[:, c:c + 128] = _as_u32(wt[:, j * 128:(j + 1) * 128])

    def load_o_weights(p):
        wcopy(3, p).wait()
        start_next(1)
        wo_s[p * PW // 2:(p + 1) * PW // 2, :] = _as_u32(stage[3, p * PW:(p + 1) * PW, :])

    def b_stages(sb):
        r0 = pl.multiple_of(sb * SEG, SEG)
        tok = yield
        if tok is not None:
            xbuf[JUNK:JUNK + 8, 0:128] = tok
        y = _layernorm(xbuf[pl.ds(r0, SEG), :])
        tok = yield
        qkv = _dot(y, _as_bf16(bq_s[...]))
        qb_s[...] = qkv[:, 0:D]
        kb_s[pl.ds(r0 + HALO, SEG), :] = qkv[:, D:2 * D]
        vb_s[pl.ds(r0 + HALO, SEG), :] = qkv[:, 2 * D:3 * D]
        pos = r0 + lax.broadcasted_iota(jnp.int32, (SEG, 128), 0)
        lg = [None] * W
        for j in range(W // 2):
            tok = yield
            if tok is not None:
                kb_s[JUNK:JUNK + 8, 0:128] = tok
            kw = kb_s[pl.ds(r0, SEG + HALO), :]
            q = qb_s[...]
            o0 = HALO - DIL * (j + W // 2)
            kj = kw[o0:o0 + SEG + 8, :]
            for w, ko in ((j, 8), (j + W // 2, 0)):
                pr = q * kj[ko:ko + SEG, :]
                t = pr[:, 0:128]
                for c in range(1, D // 128):
                    t = t + pr[:, c * 128:(c + 1) * 128]
                t = t + pltpu.roll(t, 64, 1)
                t = t + pltpu.roll(t, 32, 1)
                lg[w] = jnp.where(pos >= DIL * w, t * (scale_b * LOG2E), NEG * LOG2E)
        tok = yield
        mx = lg[0]
        for w in range(1, W):
            mx = jnp.maximum(mx, lg[w])
        es = [jnp.exp2(l - mx) for l in lg]
        den = es[0]
        for w in range(1, W):
            den = den + es[w]
        inv = 1.0 / den
        ps = [e * inv for e in es]
        acc = None
        for j in range(W // 2):
            tok = yield
            if tok is not None:
                vb_s[JUNK:JUNK + 8, 0:128] = tok
            vw = vb_s[pl.ds(r0, SEG + HALO), :]
            o0 = HALO - DIL * (j + W // 2)
            vj = vw[o0:o0 + SEG + 8, :]
            for w, ko in ((j, 8), (j + W // 2, 0)):
                pw5 = jnp.concatenate([ps[w]] * (D // 128), axis=1)
                term = pw5 * vj[ko:ko + SEG, :]
                acc = term if acc is None else acc + term
        tok = yield
        x2 = xbuf[pl.ds(r0, SEG), :] + _dot(acc, _as_bf16(bo_s[...]))
        xbuf[pl.ds(r0, SEG), :] = x2
        xio[pl.ds(r0, SEG), :] = x2.astype(xio.dtype)

    z = jnp.zeros((L, 128), F32)

    def blockdiag(a):
        a1 = a[:, 128:256]
        return jnp.concatenate([
            jnp.concatenate([a[:, 0:128], jnp.where(lo64, a1, 0.0), z], axis=1),
            jnp.concatenate([z, jnp.where(lo64, 0.0, a1), a[:, 256:384]], axis=1),
            jnp.zeros((128 - 2 * L, PW), F32)], axis=0).astype(BF16)

    sched = _make_schedule(NP)

    def step(t, mem, first=False):
        s = t if first else lax.rem(t, n_seg)
        r0 = pl.multiple_of(s * SEG, SEG)
        h = jnp.concatenate([mem, xn_s[pl.ds(r0, SEG), :]], axis=0)
        if not first:
            bgen = b_stages(lax.rem(t - 1, n_seg))
            next(bgen)
        kb, vb, qq, pr, oo = {}, {}, {}, {}, {}
        out = None
        token = None
        for op, p in sched:
            c0 = p * 9 * 128
            if op == "Pq":
                qq[p] = _dot(h, _as_bf16(w_s[:, c0:c0 + PW]))
            elif op == "Pk":
                if first:
                    load_qkv_weights(p)
                kk = _dot(h, _as_bf16(w_s[:, c0 + PW:c0 + 2 * PW]))
                token = kk[0:8, 0:128]
                kb[p] = blockdiag(kk)
            elif op == "Pv":
                vb[p] = blockdiag(_dot(h, _as_bf16(w_s[:, c0 + 2 * PW:c0 + 3 * PW])))
            elif op == "S":
                sc = _dot(qq.pop(p), kb.pop(p), _NT)
                sc = jnp.where(mask_ab, sc * (scale_a * LOG2E), fill_a)
                ma = jnp.max(jnp.where(in_a, sc, LOW), axis=-1, keepdims=True)
                mb = jnp.max(jnp.where(in_b, sc, LOW), axis=-1, keepdims=True)
                e = jnp.exp2(sc - jnp.where(in_a, ma, mb))
                la = jnp.sum(jnp.where(in_a, e, 0.0), axis=-1, keepdims=True)
                lb = jnp.sum(jnp.where(in_b, e, 0.0), axis=-1, keepdims=True)
                pr[p] = e * (1.0 / jnp.where(in_a, la, lb))
            elif op == "V":
                oo[p] = _dot(pr.pop(p), vb.pop(p))
            elif op == "O":
                if first:
                    load_o_weights(p)
                u = _dot(oo.pop(p), _as_bf16(wo_s[p * PW // 2:(p + 1) * PW // 2, :]))
                out = u if out is None else out + u
            elif op == "B":
                if not first:
                    _advance(bgen, token)
            elif op == "LN":
                rn = pl.multiple_of(lax.rem(t + 1, n_seg) * SEG, SEG)
                xbuf[JUNK:JUNK + 8, 0:128] = token
                xn_s[pl.ds(rn, SEG), :] = _layernorm(xbuf[pl.ds(rn, SEG), :])
        if not first:
            _finish(bgen)
        xbuf[pl.ds(r0, SEG), :] = xbuf[pl.ds(r0, SEG), :] + out[M:L, :]
        return out[0:M, :]

    mem_copy.wait()
    mem0 = mem_st[0:M, :].astype(F32)

    mem = step(0, mem0, first=True)
    for c in range(1, NXC):
        to_f32(c)

    def ocopy(c):
        return pltpu.make_async_copy(xio.at[pl.ds(c * XCH, XCH), :], out_hbm.at[pl.ds(c * XCH, XCH), :], sem_o.at[c])

    def loop_step(t, mem):
        mem = jnp.where(lax.rem(t, n_seg) == 0, mem0, mem)
        return step(t, mem)

    SPC = XCH // SEG

    def chunk(c, mem):
        mem = lax.fori_loop(jnp.maximum(c * SPC, 1), (c + 1) * SPC, loop_step, mem)

        @pl.when(c > NXC)
        def _():
            ocopy(c - 1 - NXC).start()
        return mem
    lax.fori_loop(0, 2 * NXC, chunk, mem)
    _finish(b_stages(n_seg - 1))
    ocopy(NXC - 1).start()
    for c in range(NXC):
        ocopy(c).wait()


@functools.partial(jax.jit, static_argnames=("A_seg_len",))
def pallas_interleave_layers__memory_aug_recurrent_mem_tr__sliding_local_dilated__prompt_kernel(
    A_x: jax.Array,
    A_mem0: jax.Array,
    A_Wq: jax.Array,
    A_Wk: jax.Array,
    A_Wv: jax.Array,
    A_Wo: jax.Array,
    A_seg_len,
    B_x: jax.Array,
    B_wqkv: jax.Array,
    B_wo: jax.Array,
):
    del B_x
    B, S, D = A_x.shape
    _, H, Dh = A_Wq.shape
    M = A_mem0.shape[1]
    SEG = int(A_seg_len)
    HB, W, DIL = 32, 8, 2
    HD = H * Dh
    kern = functools.partial(_kernel, S=S, D=D, H=H, Dh=Dh, M=M, SEG=SEG, HB=HB, W=W, DIL=DIL)
    tr = lambda w: jnp.transpose(w, (1, 2, 0)).reshape(HD, D)
    hbm = pl.BlockSpec(memory_space=pl.ANY)
    out = pl.pallas_call(
        kern,
        out_shape=jax.ShapeDtypeStruct((S, D), A_x.dtype),
        in_specs=[hbm] * 8,
        out_specs=hbm,
        scratch_shapes=[
            pltpu.VMEM((S + 32, D), F32),
            pltpu.VMEM((S, D), F32),
            pltpu.VMEM((SEG, D), F32),
            pltpu.VMEM((S + 32, D), F32),
            pltpu.VMEM((S + 32, D), F32),
            pltpu.VMEM((D // 2, 3 * D), jnp.uint32),
            pltpu.VMEM((D // 2, D), jnp.uint32),
            pltpu.VMEM((4, HD, D), BF16),
            pltpu.VMEM((D // 2, 3 * HD), jnp.uint32),
            pltpu.VMEM((HD // 2, D), jnp.uint32),
            pltpu.VMEM((S, D), A_x.dtype),
            pltpu.VMEM((D, 3 * D), BF16),
            pltpu.VMEM((D, D), BF16),
            pltpu.VMEM((64, D), BF16),
            pltpu.SemaphoreType.DMA((4, H // 2)),
            pltpu.SemaphoreType.DMA((5 + S // 512,)),
            pltpu.SemaphoreType.DMA((S // 512,)),
        ],
        compiler_params=pltpu.CompilerParams(vmem_limit_bytes=120 * 2**20),
        name="rmt_sliding",
    )(
        A_x.reshape(S, D), A_mem0.reshape(M, D),
        tr(A_Wq), tr(A_Wk), tr(A_Wv),
        A_Wo.reshape(HD, D), B_wqkv, B_wo,
    )
    return out.reshape(B, S, D)
```

```python
import functools

import jax
import jax.numpy as jnp
from jax import lax
import jax.experimental.pallas as pl
import jax.experimental.pallas.tpu as pltpu

F32 = jnp.float32
BF16 = jnp.bfloat16
NEG = -1000000000.0
LOW = -3.0e38
LOG2E = 1.4426950408889634

_NN = (((1,), (0,)), ((), ()))
_NT = (((1,), (1,)), ((), ()))


def _dot(a, b, dims=_NN):
    return lax.dot_general(a, b, dims, preferred_element_type=F32)


def _as_bf16(u):
    return pltpu.bitcast(u, BF16)


def _as_u32(b):
    return pltpu.bitcast(b, jnp.uint32)


def _layernorm(x):
    d = x.shape[-1]
    m = jnp.sum(x, axis=-1, keepdims=True) * (1.0 / d)
    xc = x - m
    v = jnp.sum(xc * xc, axis=-1, keepdims=True) * (1.0 / d)
    return xc * lax.rsqrt(v + 1e-05)


def _make_schedule(NP):
    sched = []
    bo_slot = NP - 5
    hold = (NP - 4, NP - 3)
    nxt_o = 0
    for i in range(NP):
        sched.append(("Pk", i))
        if i == 0 or 2 <= i < bo_slot:
            sched.append(("B", i))
        elif i == bo_slot + 2:
            sched.append(("LN", i))
        sched.append(("Pq", i))
        if i == 1 or i == bo_slot:
            sched.append(("B", i))
        elif i >= 2 and i not in hold:
            sched.append(("O", nxt_o))
            nxt_o += 1
        sched.append(("Pv", i))
        if i >= 1:
            sched.append(("V", i - 1))
        sched.append(("S", i))
    while nxt_o < NP - 2:
        sched.append(("O", nxt_o))
        nxt_o += 1
    sched += [("V", NP - 1), ("O", NP - 2), ("O", NP - 1)]
    return sched


def _finish(gen):
    for _ in gen:
        pass


def _advance(gen, token):
    try:
        gen.send(token)
    except StopIteration:
        pass


def _kernel(x_hbm, mem0_hbm, wqt_hbm, wkt_hbm, wvt_hbm, wo_hbm, bqkv_hbm, bwo_hbm,
            out_hbm, xbuf, xn_s, qb_s, kb_s, vb_s, bq_s, bo_s, stage, w_s, wo_s,
            xio, bq_st, bo_st, mem_st, sems, sem_b, sem_o,
            *, S, D, H, Dh, M, SEG, HB, W, DIL):
    L = M + SEG
    n_seg = S // SEG
    NP = H // 2
    PW = 2 * Dh
    DB = D // HB
    HALO = 16
    JUNK = S + HALO
    scale_a = Dh ** (-0.5)
    scale_b = DB ** (-0.5)
    XCH = 512
    NXC = S // XCH

    def wcopy(t, p):
        src = (wqt_hbm, wkt_hbm, wvt_hbm, wo_hbm)[t]
        return pltpu.make_async_copy(src.at[pl.ds(p * PW, PW), :], stage.at[t, pl.ds(p * PW, PW), :], sems.at[t, p])

    def xcopy(c):
        return pltpu.make_async_copy(x_hbm.at[pl.ds(c * XCH, XCH), :], xio.at[pl.ds(c * XCH, XCH), :], sem_b.at[5 + c])

    def bcopy(t):
        if t < 3:
            return pltpu.make_async_copy(bqkv_hbm.at[:, pl.ds(t * D, D)], bq_st.at[:, pl.ds(t * D, D)], sem_b.at[t])
        return pltpu.make_async_copy(bwo_hbm, bo_st, sem_b.at[3])

    mem_copy = pltpu.make_async_copy(mem0_hbm, mem_st.at[pl.ds(0, M), :], sem_b.at[4])

    queue = ([xcopy(0), mem_copy] + [bcopy(t) for t in range(4)]
             + [wcopy(t, p) for p in range(NP) for t in (1, 0, 2, 3)]
             + [xcopy(c) for c in range(1, NXC)])
    queue.reverse()

    def start_next(n):
        for _ in range(n):
            if queue:
                queue.pop().start()

    start_next(6)

    row = lax.broadcasted_iota(jnp.int32, (L, 128), 0)
    lane = lax.broadcasted_iota(jnp.int32, (L, 128), 1)
    key = jnp.where(lane < L, lane, lane - L)
    in_a = lane < L
    in_b = jnp.logical_and(lane >= L, lane < 2 * L)
    causal = jnp.logical_or(row < M, row >= key)
    mask_ab = jnp.logical_and(causal, lane < 2 * L)
    fill_a = jnp.where(lane < 2 * L, NEG * LOG2E, LOW)
    lo64 = lane < (Dh - 128)

    kb_s[0:HALO, :] = jnp.zeros((HALO, D), F32)
    vb_s[0:HALO, :] = jnp.zeros((HALO, D), F32)

    def to_f32(c):
        xcopy(c).wait()
        for i in range(XCH // 128):
            r = pl.multiple_of(c * XCH + i * 128, 128)
            xbuf[pl.ds(r, 128), :] = xio[pl.ds(r, 128), :].astype(F32)

    to_f32(0)
    start_next(2)
    xn_s[0:SEG, :] = _layernorm(xbuf[0:SEG, :])

    r_i = lax.broadcasted_iota(jnp.int32, (D, D), 0)
    c_i = lax.broadcasted_iota(jnp.int32, (D, D), 1)
    perm = (r_i == (c_i % HB) * DB + c_i // HB).astype(BF16)
    permT = (c_i == (r_i % HB) * DB + r_i // HB).astype(BF16)
    for t in range(3):
        bcopy(t).wait()
        start_next(3 if t == 0 else 4)
        bq_s[:, t * D:(t + 1) * D] = _as_u32(_dot(bq_st[:, t * D:(t + 1) * D], perm).astype(BF16))
    bcopy(3).wait()
    start_next(4)
    bo_s[...] = _as_u32(_dot(permT, bo_st[...]).astype(BF16))

    def load_qkv_weights(p):
        for t in (1, 0, 2):
            wcopy(t, p).wait()
            start_next(1)
            wt = stage[t, p * PW:(p + 1) * PW, :].T
            for j in range(PW // 128):
                c = (p * 9 + t * 3 + j) * 128
                w_s[:, c:c + 128] = _as_u32(wt[:, j * 128:(j + 1) * 128])

    def load_o_weights(p):
        wcopy(3, p).wait()
        start_next(1)
        wo_s[p * PW // 2:(p + 1) * PW // 2, :] = _as_u32(stage[3, p * PW:(p + 1) * PW, :])

    def b_stages(sb):
        r0 = pl.multiple_of(sb * SEG, SEG)
        tok = yield
        if tok is not None:
            xbuf[JUNK:JUNK + 8, 0:128] = tok
        y = _layernorm(xbuf[pl.ds(r0, SEG), :])
        tok = yield
        qkv = _dot(y, _as_bf16(bq_s[...]))
        qb_s[...] = qkv[:, 0:D]
        kb_s[pl.ds(r0 + HALO, SEG), :] = qkv[:, D:2 * D]
        vb_s[pl.ds(r0 + HALO, SEG), :] = qkv[:, 2 * D:3 * D]
        pos = r0 + lax.broadcasted_iota(jnp.int32, (SEG, 128), 0)
        lg = [None] * W
        for j in range(W // 2):
            tok = yield
            if tok is not None:
                kb_s[JUNK:JUNK + 8, 0:128] = tok
            kw = kb_s[pl.ds(r0, SEG + HALO), :]
            q = qb_s[...]
            o0 = HALO - DIL * (j + W // 2)
            kj = kw[o0:o0 + SEG + 8, :]
            for w, ko in ((j, 8), (j + W // 2, 0)):
                pr = q * kj[ko:ko + SEG, :]
                t = pr[:, 0:128]
                for c in range(1, D // 128):
                    t = t + pr[:, c * 128:(c + 1) * 128]
                t = t + pltpu.roll(t, 64, 1)
                t = t + pltpu.roll(t, 32, 1)
                lg[w] = jnp.where(pos >= DIL * w, t * (scale_b * LOG2E), NEG * LOG2E)
        tok = yield
        mx = lg[0]
        for w in range(1, W):
            mx = jnp.maximum(mx, lg[w])
        es = [jnp.exp2(l - mx) for l in lg]
        den = es[0]
        for w in range(1, W):
            den = den + es[w]
        inv = 1.0 / den
        ps = [e * inv for e in es]
        acc = None
        for j in range(W // 2):
            tok = yield
            if tok is not None:
                vb_s[JUNK:JUNK + 8, 0:128] = tok
            vw = vb_s[pl.ds(r0, SEG + HALO), :]
            o0 = HALO - DIL * (j + W // 2)
            vj = vw[o0:o0 + SEG + 8, :]
            for w, ko in ((j, 8), (j + W // 2, 0)):
                pw5 = jnp.concatenate([ps[w]] * (D // 128), axis=1)
                term = pw5 * vj[ko:ko + SEG, :]
                acc = term if acc is None else acc + term
        tok = yield
        x2 = xbuf[pl.ds(r0, SEG), :] + _dot(acc, _as_bf16(bo_s[...]))
        xbuf[pl.ds(r0, SEG), :] = x2
        xio[pl.ds(r0, SEG), :] = x2.astype(xio.dtype)

    z = jnp.zeros((L, 128), F32)

    def blockdiag(a):
        a1 = a[:, 128:256]
        return jnp.concatenate([
            jnp.concatenate([a[:, 0:128], jnp.where(lo64, a1, 0.0), z], axis=1),
            jnp.concatenate([z, jnp.where(lo64, 0.0, a1), a[:, 256:384]], axis=1),
            jnp.zeros((128 - 2 * L, PW), F32)], axis=0).astype(BF16)

    sched = _make_schedule(NP)

    def step(t, mem, first=False):
        s = t if first else lax.rem(t, n_seg)
        r0 = pl.multiple_of(s * SEG, SEG)
        h = jnp.concatenate([mem, xn_s[pl.ds(r0, SEG), :]], axis=0)
        if not first:
            bgen = b_stages(lax.rem(t - 1, n_seg))
            next(bgen)
        kb, vb, qq, pr, oo = {}, {}, {}, {}, {}
        out = None
        token = None
        for op, p in sched:
            c0 = p * 9 * 128
            if op == "Pq":
                qq[p] = _dot(h, _as_bf16(w_s[:, c0:c0 + PW]))
            elif op == "Pk":
                if first:
                    load_qkv_weights(p)
                kk = _dot(h, _as_bf16(w_s[:, c0 + PW:c0 + 2 * PW]))
                token = kk[0:8, 0:128]
                kb[p] = blockdiag(kk)
            elif op == "Pv":
                vb[p] = blockdiag(_dot(h, _as_bf16(w_s[:, c0 + 2 * PW:c0 + 3 * PW])))
            elif op == "S":
                sc = _dot(qq.pop(p), kb.pop(p), _NT)
                sc = jnp.where(mask_ab, sc * (scale_a * LOG2E), fill_a)
                ma = jnp.max(jnp.where(in_a, sc, LOW), axis=-1, keepdims=True)
                mb = jnp.max(jnp.where(in_b, sc, LOW), axis=-1, keepdims=True)
                e = jnp.exp2(sc - jnp.where(in_a, ma, mb))
                la = jnp.sum(jnp.where(in_a, e, 0.0), axis=-1, keepdims=True)
                lb = jnp.sum(jnp.where(in_b, e, 0.0), axis=-1, keepdims=True)
                pr[p] = e * (1.0 / jnp.where(in_a, la, lb))
            elif op == "V":
                oo[p] = _dot(pr.pop(p), vb.pop(p))
            elif op == "O":
                if first:
                    load_o_weights(p)
                u = _dot(oo.pop(p), _as_bf16(wo_s[p * PW // 2:(p + 1) * PW // 2, :]))
                out = u if out is None else out + u
            elif op == "B":
                if not first:
                    _advance(bgen, token)
            elif op == "LN":
                rn = pl.multiple_of(lax.rem(t + 1, n_seg) * SEG, SEG)
                xbuf[JUNK:JUNK + 8, 0:128] = token
                xn_s[pl.ds(rn, SEG), :] = _layernorm(xbuf[pl.ds(rn, SEG), :])
        if not first:
            _finish(bgen)
        xbuf[pl.ds(r0, SEG), :] = xbuf[pl.ds(r0, SEG), :] + out[M:L, :]
        return out[0:M, :]

    mem_copy.wait()
    mem0 = mem_st[0:M, :].astype(F32)

    mem = step(0, mem0, first=True)

    def ocopy_rows(r, n, i):
        return pltpu.make_async_copy(xio.at[pl.ds(r, n), :], out_hbm.at[pl.ds(r, n), :], sem_o.at[i])

    def ocopy(c):
        return ocopy_rows(c * XCH, XCH, c)

    def loop_step(t, mem):
        mem = jnp.where(lax.rem(t, n_seg) == 0, mem0, mem)
        return step(t, mem)

    SPC = XCH // SEG

    def chunk(c, mem):
        @pl.when(c < NXC - 1)
        def _():
            to_f32(c + 1)

        mem = lax.fori_loop(jnp.maximum(c * SPC, 1), (c + 1) * SPC, loop_step, mem)

        @pl.when(c > NXC)
        def _():
            ocopy(c - 1 - NXC).start()
        return mem
    lax.fori_loop(0, 2 * NXC, chunk, mem)
    last0 = ocopy_rows((NXC - 1) * XCH, XCH - SEG, NXC - 1)
    last1 = ocopy_rows(S - SEG, SEG, NXC)
    last0.start()
    _finish(b_stages(n_seg - 1))
    last1.start()
    for c in range(NXC - 1):
        ocopy(c).wait()
    last0.wait()
    last1.wait()


@functools.partial(jax.jit, static_argnames=("A_seg_len",))
def pallas_interleave_layers__memory_aug_recurrent_mem_tr__sliding_local_dilated__prompt_kernel(
    A_x: jax.Array,
    A_mem0: jax.Array,
    A_Wq: jax.Array,
    A_Wk: jax.Array,
    A_Wv: jax.Array,
    A_Wo: jax.Array,
    A_seg_len,
    B_x: jax.Array,
    B_wqkv: jax.Array,
    B_wo: jax.Array,
):
    del B_x
    B, S, D = A_x.shape
    _, H, Dh = A_Wq.shape
    M = A_mem0.shape[1]
    SEG = int(A_seg_len)
    HB, W, DIL = 32, 8, 2
    HD = H * Dh
    kern = functools.partial(_kernel, S=S, D=D, H=H, Dh=Dh, M=M, SEG=SEG, HB=HB, W=W, DIL=DIL)
    tr = lambda w: jnp.transpose(w, (1, 2, 0)).reshape(HD, D)
    hbm = pl.BlockSpec(memory_space=pl.ANY)
    out = pl.pallas_call(
        kern,
        out_shape=jax.ShapeDtypeStruct((S, D), A_x.dtype),
        in_specs=[hbm] * 8,
        out_specs=hbm,
        scratch_shapes=[
            pltpu.VMEM((S + 32, D), F32),
            pltpu.VMEM((S, D), F32),
            pltpu.VMEM((SEG, D), F32),
            pltpu.VMEM((S + 32, D), F32),
            pltpu.VMEM((S + 32, D), F32),
            pltpu.VMEM((D // 2, 3 * D), jnp.uint32),
            pltpu.VMEM((D // 2, D), jnp.uint32),
            pltpu.VMEM((4, HD, D), BF16),
            pltpu.VMEM((D // 2, 3 * HD), jnp.uint32),
            pltpu.VMEM((HD // 2, D), jnp.uint32),
            pltpu.VMEM((S, D), A_x.dtype),
            pltpu.VMEM((D, 3 * D), BF16),
            pltpu.VMEM((D, D), BF16),
            pltpu.VMEM((64, D), BF16),
            pltpu.SemaphoreType.DMA((4, H // 2)),
            pltpu.SemaphoreType.DMA((5 + S // 512,)),
            pltpu.SemaphoreType.DMA((S // 512 + 1,)),
        ],
        compiler_params=pltpu.CompilerParams(vmem_limit_bytes=120 * 2**20),
        name="rmt_sliding",
    )(
        A_x.reshape(S, D), A_mem0.reshape(M, D),
        tr(A_Wq), tr(A_Wk), tr(A_Wv),
        A_Wo.reshape(HD, D), B_wqkv, B_wo,
    )
    return out.reshape(B, S, D)
```

```python
import functools

import jax
import jax.numpy as jnp
from jax import lax
import jax.experimental.pallas as pl
import jax.experimental.pallas.tpu as pltpu

F32 = jnp.float32
BF16 = jnp.bfloat16
NEG = -1000000000.0
LOW = -3.0e38
LOG2E = 1.4426950408889634

_NN = (((1,), (0,)), ((), ()))
_NT = (((1,), (1,)), ((), ()))


def _dot(a, b, dims=_NN):
    return lax.dot_general(a, b, dims, preferred_element_type=F32)


def _as_bf16(u):
    return pltpu.bitcast(u, BF16)


def _as_u32(b):
    return pltpu.bitcast(b, jnp.uint32)


def _layernorm(x):
    d = x.shape[-1]
    m = jnp.sum(x, axis=-1, keepdims=True) * (1.0 / d)
    xc = x - m
    v = jnp.sum(xc * xc, axis=-1, keepdims=True) * (1.0 / d)
    return xc * lax.rsqrt(v + 1e-05)


def _make_schedule(NP):
    sched = []
    bo_slot = NP - 4
    hold = (NP - 5, NP - 2)
    nxt_o = 0
    for i in range(NP):
        sched.append(("Pk", i))
        if i == 0 or 2 <= i <= NP - 6:
            sched.append(("B", i))
        elif i == NP - 3:
            sched.append(("LN", i))
        sched.append(("Pq", i))
        if i == 1 or i == bo_slot:
            sched.append(("B", i))
        elif i >= 2 and i not in hold:
            sched.append(("O", nxt_o))
            nxt_o += 1
        sched.append(("Pv", i))
        if i >= 1:
            sched.append(("V", i - 1))
        sched.append(("S", i))
    while nxt_o < NP - 2:
        sched.append(("O", nxt_o))
        nxt_o += 1
    sched += [("V", NP - 1), ("O", NP - 2), ("O", NP - 1)]
    return sched


def _finish(gen):
    for _ in gen:
        pass


def _advance(gen, token):
    try:
        gen.send(token)
    except StopIteration:
        pass


def _kernel(x_hbm, mem0_hbm, wqt_hbm, wkt_hbm, wvt_hbm, wo_hbm, bqkv_hbm, bwo_hbm,
            out_hbm, xbuf, xn_s, qb_s, kb_s, vb_s, bq_s, bo_s, stage, w_s, wo_s,
            xio, bq_st, bo_st, mem_st, perm_s, sems, sem_b, sem_o,
            *, S, D, H, Dh, M, SEG, HB, W, DIL):
    L = M + SEG
    n_seg = S // SEG
    NP = H // 2
    PW = 2 * Dh
    DB = D // HB
    HALO = 16
    JUNK = S + HALO
    scale_a = Dh ** (-0.5)
    scale_b = DB ** (-0.5)
    XCH = 512
    NXC = S // XCH

    def wcopy(t, p):
        src = (wqt_hbm, wkt_hbm, wvt_hbm, wo_hbm)[t]
        return pltpu.make_async_copy(src.at[pl.ds(p * PW, PW), :], stage.at[t, pl.ds(p * PW, PW), :], sems.at[t, p])

    def xcopy_rows(r, n, i):
        return pltpu.make_async_copy(x_hbm.at[pl.ds(r, n), :], xio.at[pl.ds(r, n), :], sem_b.at[5 + i])

    XHEAD = 128
    xhead = xcopy_rows(0, XHEAD, NXC)
    xrest = xcopy_rows(XHEAD, XCH - XHEAD, 0)

    def xcopy(c):
        return xcopy_rows(c * XCH, XCH, c)

    def bcopy(t):
        if t < 3:
            return pltpu.make_async_copy(bqkv_hbm.at[:, pl.ds(t * D, D)], bq_st.at[:, pl.ds(t * D, D)], sem_b.at[t])
        return pltpu.make_async_copy(bwo_hbm, bo_st, sem_b.at[3])

    mem_copy = pltpu.make_async_copy(mem0_hbm, mem_st.at[pl.ds(0, M), :], sem_b.at[4])

    queue = ([xhead, mem_copy] + [bcopy(t) for t in range(4)]
             + [wcopy(t, p) for p in range(NP) for t in (1, 0, 2, 3)]
             + [xrest] + [xcopy(c) for c in range(1, NXC)])
    queue.reverse()

    def start_next(n):
        for _ in range(n):
            if queue:
                queue.pop().start()

    start_next(6)

    row = lax.broadcasted_iota(jnp.int32, (L, 128), 0)
    lane = lax.broadcasted_iota(jnp.int32, (L, 128), 1)
    key = jnp.where(lane < L, lane, lane - L)
    in_a = lane < L
    in_b = jnp.logical_and(lane >= L, lane < 2 * L)
    causal = jnp.logical_or(row < M, row >= key)
    mask_ab = jnp.logical_and(causal, lane < 2 * L)
    fill_a = jnp.where(lane < 2 * L, NEG * LOG2E, LOW)
    lo64 = lane < (Dh - 128)

    kb_s[0:HALO, :] = jnp.zeros((HALO, D), F32)
    vb_s[0:HALO, :] = jnp.zeros((HALO, D), F32)

    def to_f32(r0, n):
        for i in range(n // 128):
            r = pl.multiple_of(r0 + i * 128, 128)
            xbuf[pl.ds(r, 128), :] = xio[pl.ds(r, 128), :].astype(F32)

    xhead.wait()
    to_f32(0, XHEAD)
    start_next(2)
    xn_s[0:SEG, :] = _layernorm(xbuf[0:SEG, :])

    r_i = lax.broadcasted_iota(jnp.int32, (D, D), 0)
    c_i = lax.broadcasted_iota(jnp.int32, (D, D), 1)
    perm_s[0] = _as_u32((r_i == (c_i % HB) * DB + c_i // HB).astype(BF16))
    perm_s[1] = _as_u32((c_i == (r_i % HB) * DB + r_i // HB).astype(BF16))
    for t in range(3):
        bcopy(t).wait()
        start_next(3 if t == 0 else 4)

        def perm_rows(i, _, t=t):
            r = pl.multiple_of(i * 128, 128)
            w = _dot(bq_st[pl.ds(r, 128), t * D:(t + 1) * D], _as_bf16(perm_s[0]))
            bq_s[pl.ds(pl.multiple_of(i * 64, 64), 64), t * D:(t + 1) * D] = _as_u32(w.astype(BF16))
            return 0
        lax.fori_loop(0, D // 128, perm_rows, 0)
    bcopy(3).wait()
    start_next(4)

    def perm_o_rows(i, _):
        pt = _as_bf16(perm_s[1, pl.ds(pl.multiple_of(i * 64, 64), 64), :])
        bo_s[pl.ds(pl.multiple_of(i * 64, 64), 64), :] = _as_u32(_dot(pt, bo_st[...]).astype(BF16))
        return 0
    lax.fori_loop(0, D // 128, perm_o_rows, 0)

    def load_qkv_weights(p):
        for t in (1, 0, 2):
            wcopy(t, p).wait()
            start_next(1)
            wt = stage[t, p * PW:(p + 1) * PW, :].T
            for j in range(PW // 128):
                c = (p * 9 + t * 3 + j) * 128
                w_s[:, c:c + 128] = _as_u32(wt[:, j * 128:(j + 1) * 128])

    def load_o_weights(p):
        wcopy(3, p).wait()
        start_next(1)
        wo_s[p * PW // 2:(p + 1) * PW // 2, :] = _as_u32(stage[3, p * PW:(p + 1) * PW, :])

    def b_stages(sb):
        r0 = pl.multiple_of(sb * SEG, SEG)
        tok = yield
        if tok is not None:
            xbuf[JUNK:JUNK + 8, 0:128] = tok
        y = _layernorm(xbuf[pl.ds(r0, SEG), :])
        tok = yield
        qkv = _dot(y, _as_bf16(bq_s[...]))
        qb_s[...] = qkv[:, 0:D]
        kb_s[pl.ds(r0 + HALO, SEG), :] = qkv[:, D:2 * D]
        vb_s[pl.ds(r0 + HALO, SEG), :] = qkv[:, 2 * D:3 * D]
        pos = r0 + lax.broadcasted_iota(jnp.int32, (SEG, 128), 0)
        lg = [None] * W
        for j in range(W // 2):
            tok = yield
            if tok is not None:
                kb_s[JUNK:JUNK + 8, 0:128] = tok
            kw = kb_s[pl.ds(r0, SEG + HALO), :]
            q = qb_s[...]
            o0 = HALO - DIL * (j + W // 2)
            kj = kw[o0:o0 + SEG + 8, :]
            for w, ko in ((j, 8), (j + W // 2, 0)):
                pr = q * kj[ko:ko + SEG, :]
                t = pr[:, 0:128]
                for c in range(1, D // 128):
                    t = t + pr[:, c * 128:(c + 1) * 128]
                t = t + pltpu.roll(t, 64, 1)
                t = t + pltpu.roll(t, 32, 1)
                lg[w] = jnp.where(pos >= DIL * w, t * (scale_b * LOG2E), NEG * LOG2E)
        tok = yield
        mx = lg[0]
        for w in range(1, W):
            mx = jnp.maximum(mx, lg[w])
        es = [jnp.exp2(l - mx) for l in lg]
        den = es[0]
        for w in range(1, W):
            den = den + es[w]
        inv = 1.0 / den
        ps = [e * inv for e in es]
        acc = None
        for j in range(W // 2):
            tok = yield
            if tok is not None:
                vb_s[JUNK:JUNK + 8, 0:128] = tok
            vw = vb_s[pl.ds(r0, SEG + HALO), :]
            o0 = HALO - DIL * (j + W // 2)
            vj = vw[o0:o0 + SEG + 8, :]
            for w, ko in ((j, 8), (j + W // 2, 0)):
                pw5 = jnp.concatenate([ps[w]] * (D // 128), axis=1)
                term = pw5 * vj[ko:ko + SEG, :]
                acc = term if acc is None else acc + term
        tok = yield
        x2 = xbuf[pl.ds(r0, SEG), :] + _dot(acc, _as_bf16(bo_s[...]))
        xbuf[pl.ds(r0, SEG), :] = x2
        xio[pl.ds(r0, SEG), :] = x2.astype(xio.dtype)

    z = jnp.zeros((L, 128), F32)

    def blockdiag(a):
        a1 = a[:, 128:256]
        return jnp.concatenate([
            jnp.concatenate([a[:, 0:128], jnp.where(lo64, a1, 0.0), z], axis=1),
            jnp.concatenate([z, jnp.where(lo64, 0.0, a1), a[:, 256:384]], axis=1),
            jnp.zeros((128 - 2 * L, PW), F32)], axis=0).astype(BF16)

    sched = _make_schedule(NP)

    def step(t, mem, first=False):
        s = t if first else lax.rem(t, n_seg)
        r0 = pl.multiple_of(s * SEG, SEG)
        h = jnp.concatenate([mem, xn_s[pl.ds(r0, SEG), :]], axis=0)
        if not first:
            bgen = b_stages(lax.rem(t - 1, n_seg))
            next(bgen)
        kb, vb, qq, pr, oo = {}, {}, {}, {}, {}
        out = None
        token = None
        for op, p in sched:
            c0 = p * 9 * 128
            if op == "Pq":
                qq[p] = _dot(h, _as_bf16(w_s[:, c0:c0 + PW]))
            elif op == "Pk":
                if first:
                    load_qkv_weights(p)
                kk = _dot(h, _as_bf16(w_s[:, c0 + PW:c0 + 2 * PW]))
                token = kk[L - 8:L, 128:256]
                kb[p] = blockdiag(kk)
            elif op == "Pv":
                vb[p] = blockdiag(_dot(h, _as_bf16(w_s[:, c0 + 2 * PW:c0 + 3 * PW])))
            elif op == "S":
                sc = _dot(qq.pop(p), kb.pop(p), _NT)
                sc = jnp.where(mask_ab, sc * (scale_a * LOG2E), fill_a)
                ma = jnp.max(jnp.where(in_a, sc, LOW), axis=-1, keepdims=True)
                mb = jnp.max(jnp.where(in_b, sc, LOW), axis=-1, keepdims=True)
                e = jnp.exp2(sc - jnp.where(in_a, ma, mb))
                la = jnp.sum(jnp.where(in_a, e, 0.0), axis=-1, keepdims=True)
                lb = jnp.sum(jnp.where(in_b, e, 0.0), axis=-1, keepdims=True)
                pr[p] = e * (1.0 / jnp.where(in_a, la, lb))
            elif op == "V":
                oo[p] = _dot(pr.pop(p), vb.pop(p))
            elif op == "O":
                if first:
                    load_o_weights(p)
                u = _dot(oo.pop(p), _as_bf16(wo_s[p * PW // 2:(p + 1) * PW // 2, :]))
                out = u if out is None else out + u
            elif op == "B":
                if not first:
                    _advance(bgen, token)
            elif op == "LN":
                rn = pl.multiple_of(lax.rem(t + 1, n_seg) * SEG, SEG)
                xbuf[JUNK:JUNK + 8, 0:128] = token
                xn_s[pl.ds(rn, SEG), :] = _layernorm(xbuf[pl.ds(rn, SEG), :])
        if not first:
            _finish(bgen)
        xbuf[pl.ds(r0, SEG), :] = xbuf[pl.ds(r0, SEG), :] + out[M:L, :]
        return out[0:M, :]

    mem_copy.wait()
    mem0 = mem_st[0:M, :].astype(F32)

    mem = step(0, mem0, first=True)
    xrest.wait()
    to_f32(XHEAD, XCH - XHEAD)

    def ocopy_rows(r, n, i):
        return pltpu.make_async_copy(xio.at[pl.ds(r, n), :], out_hbm.at[pl.ds(r, n), :], sem_o.at[i])

    def ocopy(c):
        return ocopy_rows(c * XCH, XCH, c)

    def loop_step(t, mem):
        mem = jnp.where(lax.rem(t, n_seg) == 0, mem0, mem)
        return step(t, mem)

    SPC = XCH // SEG

    def chunk(c, mem):
        @pl.when(c < NXC - 1)
        def _():
            xcopy(c + 1).wait()
            to_f32((c + 1) * XCH, XCH)

        mem = lax.fori_loop(jnp.maximum(c * SPC, 1), (c + 1) * SPC, loop_step, mem)

        @pl.when(c > NXC)
        def _():
            ocopy(c - 1 - NXC).start()
        return mem
    lax.fori_loop(0, 2 * NXC, chunk, mem)
    last0 = ocopy_rows((NXC - 1) * XCH, XCH - SEG, NXC - 1)
    last1 = ocopy_rows(S - SEG, SEG, NXC)
    last0.start()
    _finish(b_stages(n_seg - 1))
    last1.start()
    for c in range(NXC - 1):
        ocopy(c).wait()
    last0.wait()
    last1.wait()


@functools.partial(jax.jit, static_argnames=("A_seg_len",))
def pallas_interleave_layers__memory_aug_recurrent_mem_tr__sliding_local_dilated__prompt_kernel(
    A_x: jax.Array,
    A_mem0: jax.Array,
    A_Wq: jax.Array,
    A_Wk: jax.Array,
    A_Wv: jax.Array,
    A_Wo: jax.Array,
    A_seg_len,
    B_x: jax.Array,
    B_wqkv: jax.Array,
    B_wo: jax.Array,
):
    del B_x
    B, S, D = A_x.shape
    _, H, Dh = A_Wq.shape
    M = A_mem0.shape[1]
    SEG = int(A_seg_len)
    HB, W, DIL = 32, 8, 2
    HD = H * Dh
    kern = functools.partial(_kernel, S=S, D=D, H=H, Dh=Dh, M=M, SEG=SEG, HB=HB, W=W, DIL=DIL)
    tr = lambda w: jnp.transpose(w, (1, 2, 0)).reshape(HD, D)
    hbm = pl.BlockSpec(memory_space=pl.ANY)
    out = pl.pallas_call(
        kern,
        out_shape=jax.ShapeDtypeStruct((S, D), A_x.dtype),
        in_specs=[hbm] * 8,
        out_specs=hbm,
        scratch_shapes=[
            pltpu.VMEM((S + 32, D), F32),
            pltpu.VMEM((S, D), F32),
            pltpu.VMEM((SEG, D), F32),
            pltpu.VMEM((S + 32, D), F32),
            pltpu.VMEM((S + 32, D), F32),
            pltpu.VMEM((D // 2, 3 * D), jnp.uint32),
            pltpu.VMEM((D // 2, D), jnp.uint32),
            pltpu.VMEM((4, HD, D), BF16),
            pltpu.VMEM((D // 2, 3 * HD), jnp.uint32),
            pltpu.VMEM((HD // 2, D), jnp.uint32),
            pltpu.VMEM((S, D), A_x.dtype),
            pltpu.VMEM((D, 3 * D), BF16),
            pltpu.VMEM((D, D), BF16),
            pltpu.VMEM((64, D), BF16),
            pltpu.VMEM((2, D // 2, D), jnp.uint32),
            pltpu.SemaphoreType.DMA((4, H // 2)),
            pltpu.SemaphoreType.DMA((6 + S // 512,)),
            pltpu.SemaphoreType.DMA((S // 512 + 1,)),
        ],
        compiler_params=pltpu.CompilerParams(vmem_limit_bytes=120 * 2**20),
        name="rmt_sliding",
    )(
        A_x.reshape(S, D), A_mem0.reshape(M, D),
        tr(A_Wq), tr(A_Wk), tr(A_Wv),
        A_Wo.reshape(HD, D), B_wqkv, B_wo,
    )
    return out.reshape(B, S, D)
```
